```python
import os as _os
_os.environ.setdefault("JAX_PLATFORMS", "cpu")
import jax
import jax.numpy as jnp

def _softmax(x, axis=-1):
    return jax.nn.softmax(x, axis=axis)
def _gelu(x):
    return jax.nn.gelu(x, approximate=True)
def _silu(x):
    return jax.nn.silu(x)
def _sigmoid(x):
    return jax.nn.sigmoid(x)
def _layernorm(x, axis=-1, eps=1e-5):
    m = jnp.mean(x, axis=axis, keepdims=True)
    v = jnp.var(x, axis=axis, keepdims=True)
    return (x - m) / jnp.sqrt(v + eps)
def _scatter_add(tgt, idx, src, axis=0):
    return tgt.at[idx].add(src)
def _segment_sum(src, seg, n):
    return jax.ops.segment_sum(src, seg, n)
class _Rng:
    def __init__(self, key):
        self._k = key
    def _next(self):
        self._k, sub = jax.random.split(self._k)
        return sub
    def normal(self, shape):
        return jax.random.normal(self._next(), shape, dtype=jnp.bfloat16)
    def randint(self, lo, hi, shape):
        return jax.random.randint(self._next(), shape, lo, hi, dtype=jnp.int32)
    def uniform(self, shape, lo=0.0, hi=1.0):
        return jax.random.uniform(self._next(), shape, jnp.bfloat16, lo, hi)
    def permutation(self, n):
        return jax.random.permutation(self._next(), n)


kernel_name = 'concat_heads__softmax_full_mha__ssm_conv_s5__prompt'

def setup_inputs():
    _rng = _Rng(jax.random.key(int.from_bytes(__import__("os").urandom(4), "little")))
    _w = (lambda a: (lambda t: t.astype(jnp.bfloat16) if jnp.issubdtype(t.dtype, jnp.floating) else t)(jnp.asarray(a)))
    def _A_setup():
        B, S, D = 1, 2048, 512
        return {
            "x": _w((lambda *s: _rng.normal(s) * 0.2)(B, S, D)),
            "wqkv": _w((lambda *s: _rng.normal(s) * 0.2)(D, 3 * D)),
            "wo": _w((lambda *s: _rng.normal(s) * 0.05)(D, D)),
        }
    _A_in = _A_setup()

    def _B_setup():
        B, S, D = 1, 2048, 512
        P = D
        Lambda_re = -0.5 * jnp.exp((lambda *s: _rng.normal(s) * 0.4)(P))
        Lambda_im = (lambda *s: _rng.normal(s) * 0.4)(P) * 1.0
        B_re = (lambda *s: _rng.normal(s) * 0.4)(P, D) * (D ** -0.5)
        B_im = (lambda *s: _rng.normal(s) * 0.4)(P, D) * (D ** -0.5)
        C_re = (lambda *s: _rng.normal(s) * 0.4)(D, P) * (P ** -0.5)
        C_im = (lambda *s: _rng.normal(s) * 0.4)(D, P) * (P ** -0.5)
        log_dt = (lambda *s: _rng.normal(s) * 0.4)(P) * 0.3 - 2.0
        Dskip = (lambda *s: _rng.normal(s) * 0.4)(D)
        return {
            "x": _w((lambda *s: _rng.normal(s) * 0.05)(B, S, D)),
            "Lambda_re": _w(Lambda_re),
            "Lambda_im": _w(Lambda_im),
            "B_re": _w(B_re),
            "B_im": _w(B_im),
            "C_re": _w(C_re),
            "C_im": _w(C_im),
            "log_dt": _w(log_dt),
            "Dskip": _w(Dskip),
        }
    _B_in = _B_setup()

    return {
        "A_x": _A_in["x"],
        "A_wqkv": _A_in["wqkv"],
        "A_wo": _A_in["wo"],
        "B_x": _B_in["x"],
        "B_Lambda_re": _B_in["Lambda_re"],
        "B_Lambda_im": _B_in["Lambda_im"],
        "B_B_re": _B_in["B_re"],
        "B_B_im": _B_in["B_im"],
        "B_C_re": _B_in["C_re"],
        "B_C_im": _B_in["C_im"],
        "B_log_dt": _B_in["log_dt"],
        "B_Dskip": _B_in["Dskip"],
    }

def reference(A_x, A_wqkv, A_wo, B_x, B_Lambda_re, B_Lambda_im, B_B_re, B_B_im, B_C_re, B_C_im, B_log_dt, B_Dskip):
    def _A_ref(x, wqkv, wo):
        B, S, D = x.shape
        H = 32; Dh = D // H
        qkv = (lambda x, *d: x.transpose(*d))((x @ wqkv).reshape(B, S, 3, H, Dh), 2, 0, 3, 1, 4)
        q, k, v = qkv[0], qkv[1], qkv[2]
        scale = Dh ** -0.5
        scores = jnp.einsum("bhqd,bhkd->bhqk", q, k) * scale
        p = _softmax(scores, axis=-1)
        o = jnp.einsum("bhqk,bhkd->bhqd", p, v)
        return (lambda x, *d: x.transpose(*d))(o, 0, 2, 1, 3).reshape(B, S, D) @ wo

    def _B_ref(x, Lambda_re, Lambda_im, B_re, B_im, C_re, C_im, log_dt, Dskip):
        Bsz, L, H = x.shape
        Lam = Lambda_re + 1j * Lambda_im
        Bmat = B_re + 1j * B_im
        Cmat = C_re + 1j * C_im
        dt = jnp.exp(log_dt)
        Lam_bar = jnp.exp(dt * Lam)
        B_bar = ((Lam_bar - 1.0) / Lam)[:, None] * Bmat
        Bu = jnp.einsum("bld,pd->blp", x + 0j, B_bar)
        h = jnp.zeros_like(Bu[:, 0, :])
        hs = []
        for t in range(L):
            h = Lam_bar[None, :] * h + Bu[:, t, :]
            hs.append(h)
        hseq = jnp.stack(hs, 1)
        y = 2.0 * jnp.einsum("blp,dp->bld", hseq, Cmat).real + x * Dskip[None, None, :]
        return y

    a = _A_ref(A_x, A_wqkv, A_wo)
    b = _B_ref(B_x, B_Lambda_re, B_Lambda_im, B_B_re, B_B_im, B_C_re, B_C_im, B_log_dt, B_Dskip)
    return jnp.concatenate([a, b], axis=-1)
```

```python
import math

import jax
import jax.numpy as jnp
import jax.experimental.pallas as pl
import jax.experimental.pallas.tpu as pltpu

F32 = jnp.float32
BF16 = jnp.bfloat16

S = 2048
D = 512
H = 32
DH = 16
P = 512
TQ = 512
KC = 128
NC = S // KC
NQ = S // TQ
N = NQ * H
UNR = 8
SKEW = 2
TIE = 4
TIE_EVERY = 3
VR = 16
VPU_CHUNKS = [c for c in range(NC) if c % 4 != 0]
L_LO = 2.0 ** -30
L_HI = 2.0 ** 70
F32_MAX = 3.0e38
RC = 128
QSCALE = (DH ** -0.5) * math.log2(math.e)


def _vpu_schedule(shift=0.7):
    halves = [(c, hf) for c in VPU_CHUNKS for hf in range(2)]
    sched = {c: [] for c in range(NC)}
    for k, (c, hf) in enumerate(halves):
        x = min((k + shift) * NC / len(halves), c + 0.99)
        item = int(x)
        groups = (KC - VR if item in VPU_CHUNKS else KC) // 8
        sched[item].append((min(int((x - item) * groups), groups - 1), c, hf))
    return sched


VPU_SCHED = _vpu_schedule()
PEND_KEYS = [(c, hf) for item in range(SKEW) for (_, c, hf) in VPU_SCHED[item] if c >= SKEW]

_NT = (((1,), (1,)), ((), ()))
_TN = (((0,), (0,)), ((), ()))


def _dot(a, b):
    return jnp.dot(a, b, preferred_element_type=F32)


def _make_w(qt_ref, qf_ref, n, j, slot, fill=True):
    n = jnp.minimum(n, N - 1)
    t = n // H
    h = n % H
    q = qt_ref[pl.ds(pl.multiple_of(h * DH, DH), DH), pl.ds(pl.multiple_of(t * TQ, TQ), TQ)]
    if fill:
        qf_ref[slot] = q.astype(F32)
    parts = []
    if j > 0:
        parts.append(jnp.zeros((DH * j, TQ), BF16))
    parts.append(q)
    if j < 7:
        parts.append(jnp.zeros((DH * (7 - j), TQ), BF16))
    return jnp.concatenate(parts, axis=0), h // 8, j


def _vpu_scores(kf_ref, qf_ref, g, j, slot, c, half):
    kg = kf_ref[g, VPU_CHUNKS.index(c), 8 * half:8 * half + 8, :]
    kb = [jnp.broadcast_to(kg[:, DH * j + d:DH * j + d + 1], (8, 128)) for d in range(DH)]
    outs = []
    for lt in range(TQ // 128):
        acc = None
        for d in range(DH):
            qrow = qf_ref[slot, d:d + 1, 128 * lt:128 * (lt + 1)]
            term = kb[d] * jnp.broadcast_to(qrow, (8, 128))
            acc = term if acc is None else acc + term
        outs.append(acc)
    return jnp.concatenate(outs, axis=1)


def _exp_item(k_ref, kf_ref, qf_ref, wgj, slot, c, lsum, pend):
    w, g, j = wgj
    nm = KC - VR if c in VPU_CHUNKS else KC
    p = jnp.exp2(_dot(k_ref[g, pl.ds(c * KC, nm), :], w))
    rows = [p[8 * r:8 * r + 8, :] for r in range(nm // 8)]
    for r in range(nm // 8):
        lsum = rows[r] if lsum is None else lsum + rows[r]
        for (rr, cc, half) in VPU_SCHED[c]:
            if rr == r:
                pend[cc, half] = jnp.exp2(_vpu_scores(kf_ref, qf_ref, g, j, slot, cc, half))
                lsum = lsum + pend[cc, half]
    if c in VPU_CHUNKS:
        rows = rows + [pend.pop((c, 0)), pend.pop((c, 1))]
    return jnp.concatenate(rows, axis=0).astype(BF16), lsum


def _cmul(ar, ai, br, bi):
    return ar * br - ai * bi, ar * bi + ai * br


def _kernel(xa_hbm, wqkv_hbm, wo_hbm, xb_hbm, lre_hbm, lim_hbm, bre_hbm, bim_hbm,
            cre_hbm, cim_hbm, ldt_hbm, dsk_hbm,
            o_hbm,
            xa_ref, wq_ref, wk_ref, wv_ref, wo_ref, xb_ref, bre_ref, bim_ref, cre_ref, cim_ref,
            sems,
            qt_ref, k_ref, vt_ref, pc_ref, ls_ref, pd_ref, ok_ref, ot_ref,
            pw_ref, u_ref, carry_ref,
            lre_ref, lim_ref, ldt_ref, dsk_ref, o_ref, osems, wqt_ref, wvt_ref, acc_ref, kf_ref, qf_ref):
    t = pl.program_id(0)

    copies = [
        (lre_hbm, lre_ref), (lim_hbm, lim_ref), (ldt_hbm, ldt_ref), (dsk_hbm, dsk_ref),
        (wqkv_hbm.at[:, D:2 * D], wk_ref),
        (xa_hbm.at[0:TQ, :], xa_ref.at[0:TQ, :]),
        (xa_hbm.at[TQ:2 * TQ, :], xa_ref.at[TQ:2 * TQ, :]),
        (xa_hbm.at[2 * TQ:S, :], xa_ref.at[2 * TQ:S, :]),
        (wqkv_hbm.at[:, 0:D], wq_ref),
        (wqkv_hbm.at[:, 2 * D:3 * D], wv_ref),
        (bre_hbm, bre_ref), (bim_hbm, bim_ref), (cre_hbm, cre_ref), (cim_hbm, cim_ref),
        (xb_hbm, xb_ref), (wo_hbm, wo_ref),
    ]
    dmas = [pltpu.make_async_copy(src, dst, sems.at[i]) for i, (src, dst) in enumerate(copies)]

    @pl.when(t == 0)
    def _():
        for d in dmas:
            d.start()
        for d in dmas[0:4]:
            d.wait()

        lre = lre_ref[...].astype(F32).reshape(1, P)
        lim = lim_ref[...].astype(F32).reshape(1, P)
        dt = jnp.exp(ldt_ref[...].astype(F32).reshape(1, P)).astype(BF16).astype(F32)
        mag = jnp.exp(dt * lre)
        ar = mag * jnp.cos(dt * lim)
        ai = mag * jnp.sin(dt * lim)
        den = lre * lre + lim * lim
        cr = ((ar - 1.0) * lre + ai * lim) / den
        ci = (ai * lre - (ar - 1.0) * lim) / den
        a1 = (ar, ai)
        a2 = _cmul(*a1, *a1)
        a3 = _cmul(*a2, *a1)
        a4 = _cmul(*a2, *a2)
        a5 = _cmul(*a4, *a1)
        a6 = _cmul(*a4, *a2)
        a7 = _cmul(*a4, *a3)
        a8 = _cmul(*a4, *a4)
        row = jax.lax.broadcasted_iota(jnp.int32, (8, P), 0)
        for idx, (a, sh) in enumerate(((a1, 1), (a2, 2), (a4, 4))):
            for part in range(2):
                pw_ref[2 * idx + part] = jnp.where(
                    row >= sh, jnp.broadcast_to(a[part], (8, P)), 0.0)
        for part in range(2):
            pw_ref[6 + part] = jnp.concatenate(
                [a[part] for a in (a1, a2, a3, a4, a5, a6, a7, a8)], axis=0)
        pw_ref[8] = jnp.broadcast_to(2.0 * cr, (8, P))
        pw_ref[9] = jnp.broadcast_to(2.0 * ci, (8, P))
        carry_ref[...] = jnp.zeros_like(carry_ref)

        def project_k(r0, r1):
            kk = _dot(xa_ref[r0:r1, :], wk_ref[...]).astype(BF16)
            for g in range(4):
                k_ref[g, r0:r1, :] = kk[:, 128 * g:128 * (g + 1)]
                for c in range(r0 // KC, r1 // KC):
                    if c in VPU_CHUNKS:
                        rows = slice((c + 1) * KC - VR - r0, (c + 1) * KC - r0)
                        kf_ref[g, VPU_CHUNKS.index(c)] = kk[rows, 128 * g:128 * (g + 1)].astype(F32)

        dmas[4].wait()
        dmas[5].wait()
        project_k(0, TQ)
        dmas[6].wait()
        project_k(TQ, 2 * TQ)
        dmas[7].wait()
        dmas[8].wait()
        project_k(2 * TQ, S)
        wqt_ref[...] = wq_ref[...].T
        dmas[9].wait()
        qt = jax.lax.dot_general(wqt_ref[...], xa_ref[...], _NT, preferred_element_type=F32)
        qt_ref[...] = (qt * QSCALE).astype(BF16)
        wvt_ref[...] = wv_ref[...].T
        vt = jax.lax.dot_general(wvt_ref[...], xa_ref[...], _NT, preferred_element_type=F32)
        vt_ref[...] = vt.astype(BF16)
        wgj = _make_w(qt_ref, qf_ref, 0, 0, 0)
        lsum = None
        pend = {}
        for c in range(SKEW):
            pc_ref[c], lsum = _exp_item(k_ref, kf_ref, qf_ref, wgj, 0, c, lsum, pend)
        ls_ref[...] = lsum
        for k, key in enumerate(PEND_KEYS):
            pd_ref[k] = pend.pop(key)
        assert not pend
        for d in dmas[10:]:
            d.wait()

    ok_ref[...] = jnp.ones_like(ok_ref)

    def body(b, carry):
        n0 = t * H + b * UNR
        wgj = _make_w(qt_ref, qf_ref, n0, 0, 0, fill=False)
        lsum = ls_ref[...]
        pend = {key: pd_ref[k] for k, key in enumerate(PEND_KEYS)}
        pt = {c: pc_ref[c] for c in range(SKEW)}
        ls_hist = {SKEW - 1: lsum}
        inv = {}
        ni = UNR * NC
        for i in range(ni):
            e = i + SKEW
            es, ec = e // NC, e % NC
            if ec == 0:
                wgj = _make_w(qt_ref, qf_ref, n0 + es, es % 8, es % 2)
                lsum = None
            pt[e], lsum = _exp_item(k_ref, kf_ref, qf_ref, wgj, es % 2, ec, lsum, pend)
            ls_hist[e] = lsum
            if ec == NC - 1:
                l = jnp.sum(lsum, axis=0, keepdims=True)
                inv[es] = 1.0 / l
                safe = jnp.logical_and(l >= L_LO, l <= L_HI)
                ok_ref[...] = jnp.where(safe, ok_ref[...], 0.0)
            ps, pc = i // NC, i % NC
            h = b * UNR + ps
            vt = vt_ref[pl.ds(pl.multiple_of(h * DH, DH), DH), pl.ds(pc * KC, KC)]
            if i % TIE_EVERY == TIE_EVERY - 1:
                lo = ls_hist[max(e - TIE, SKEW - 1)]
                z = (lo[:, 0:128] + lo[:, 128:256]) + (lo[:, 256:384] + lo[:, 384:512])
                z = jnp.minimum(z, 0.0)
                vt = (vt.astype(F32) + jnp.concatenate([z, z], axis=0)).astype(BF16)
            d = _dot(vt, pt.pop(i))
            if pc == 0:
                acc_ref[...] = d
            elif pc < NC - 1:
                acc_ref[...] = acc_ref[...] + d
            else:
                o = (acc_ref[...] + d) * inv[ps]
                fin = jnp.abs(o) <= F32_MAX
                ok_ref[...] = jnp.where(jnp.logical_and(fin[0:8, :], fin[8:16, :]),
                                        ok_ref[...], 0.0)
                ot_ref[pl.ds(pl.multiple_of(h * DH, DH), DH), :] = o.astype(BF16)
        for c in range(SKEW):
            pc_ref[c] = pt[ni + c]
        ls_ref[...] = lsum
        for k, key in enumerate(PEND_KEYS):
            pd_ref[k] = pend.pop(key)
        assert not pend
        return carry

    jax.lax.fori_loop(0, H // UNR, body, 0)

    row0 = pl.multiple_of(t * TQ, TQ)

    def u_chunk(c):
        xb = xb_ref[pl.ds(row0 + c * RC, RC), :]
        rows = slice(c * RC, (c + 1) * RC)
        u_ref[rows, 0:P] = jax.lax.dot_general(xb, bre_ref[...], _NT, preferred_element_type=F32)
        u_ref[rows, P:2 * P] = jax.lax.dot_general(xb, bim_ref[...], _NT, preferred_element_type=F32)

    def scan_chunk(c, cr, ci, last):
        nt = P // 128
        crs = [cr[:, 128 * j:128 * (j + 1)] for j in range(nt)]
        cis = [ci[:, 128 * j:128 * (j + 1)] for j in range(nt)]
        for i in range(RC // 8):
            rows = slice(c * RC + i * 8, c * RC + i * 8 + 8)
            for j in range(nt):
                lre_ = slice(128 * j, 128 * (j + 1))
                lim_ = slice(P + 128 * j, P + 128 * (j + 1))
                yr = u_ref[rows, lre_]
                yi = u_ref[rows, lim_]
                if last is not None:
                    yr = yr + jnp.minimum(jnp.maximum(last, 0.0), 0.0)
                for idx, sh in enumerate((1, 2, 4)):
                    sr = pltpu.roll(yr, sh, 0)
                    si = pltpu.roll(yi, sh, 0)
                    pr, pi = _cmul(pw_ref[2 * idx, :, lre_], pw_ref[2 * idx + 1, :, lre_], sr, si)
                    yr, yi = yr + pr, yi + pi
                pr, pi = _cmul(pw_ref[6, :, lre_], pw_ref[7, :, lre_], crs[j], cis[j])
                gr, gi = yr + pr, yi + pi
                c2r, c2i = pw_ref[8, :, lre_], pw_ref[9, :, lre_]
                u_ref[rows, lre_] = gr * c2r - gi * c2i
                u_ref[rows, lim_] = -(gr * c2i) - gi * c2r
                crs[j] = jnp.broadcast_to(gr[7:8, :], (8, 128))
                cis[j] = jnp.broadcast_to(gi[7:8, :], (8, 128))
                last = gr
        return jnp.concatenate(crs, axis=1), jnp.concatenate(cis, axis=1), last

    def out_dma(c, half, r0):
        cols = slice(half * D, (half + 1) * D)
        return pltpu.make_async_copy(o_ref.at[c * RC:(c + 1) * RC, cols],
                                     o_hbm.at[pl.ds(r0 + c * RC, RC), cols],
                                     osems.at[2 * c + half])

    def y_chunk(c):
        rows = slice(c * RC, (c + 1) * RC)
        y = (jax.lax.dot_general(u_ref[rows, 0:P].astype(BF16), cre_ref[...], _NT,
                                 preferred_element_type=F32)
             + jax.lax.dot_general(u_ref[rows, P:2 * P].astype(BF16), cim_ref[...], _NT,
                                   preferred_element_type=F32))
        xb = xb_ref[pl.ds(row0 + c * RC, RC), :].astype(F32)
        o_ref[rows, D:2 * D] = y + xb * dsk_ref[...].astype(F32).reshape(1, D)
        out_dma(c, 1, row0).start()

    def a_chunk(c):
        rows = slice(c * RC, (c + 1) * RC)
        o_ref[rows, 0:D] = jax.lax.dot_general(ot_ref[:, rows], wo_ref[...], _TN,
                                               preferred_element_type=F32)
        out_dma(c, 0, row0).start()

    nch = TQ // RC

    def wait_out(r0):
        for c in range(nch):
            for half in range(2):
                out_dma(c, half, r0).wait()

    @pl.when(t > 0)
    def _():
        wait_out(pl.multiple_of((t - 1) * TQ, TQ))

    cr, ci = carry_ref[0], carry_ref[1]
    last = None
    u_chunk(0)
    for c in range(nch):
        if c + 1 < nch:
            u_chunk(c + 1)
        a_chunk(c)
        cr, ci, last = scan_chunk(c, cr, ci, last)
        if c > 0:
            y_chunk(c - 1)
    y_chunk(nch - 1)
    carry_ref[0] = cr
    carry_ref[1] = ci
    unsafe = jnp.min(ok_ref[...]) < 0.5

    @pl.when(unsafe)
    def _():
        for c in range(nch):
            out_dma(c, 0, row0).wait()

        def head(h, carry):
            g = h // 8
            qg = qt_ref[pl.ds(pl.multiple_of(g * 128, 128), 128),
                        pl.ds(pl.multiple_of(t * TQ, TQ), TQ)]
            row = jax.lax.broadcasted_iota(jnp.int32, (128, TQ), 0)
            w = jnp.where((row // DH) == h % 8, qg, jnp.zeros_like(qg))

            def scores(c):
                return _dot(k_ref[g, pl.ds(pl.multiple_of(c * KC, KC), KC), :], w)

            def row_max(c, m):
                return jnp.maximum(m, jnp.max(scores(c), axis=0, keepdims=True))

            m = jax.lax.fori_loop(0, NC, row_max, jnp.full((1, TQ), -jnp.inf, F32))

            def accumulate(c, la):
                l, acc = la
                p = jnp.exp2(scores(c) - m)
                vt = vt_ref[pl.ds(pl.multiple_of(h * DH, DH), DH),
                            pl.ds(pl.multiple_of(c * KC, KC), KC)]
                return l + jnp.sum(p, axis=0, keepdims=True), acc + _dot(vt, p.astype(BF16))

            l, acc = jax.lax.fori_loop(
                0, NC, accumulate, (jnp.zeros((1, TQ), F32), jnp.zeros((DH, TQ), F32)))
            ot_ref[pl.ds(pl.multiple_of(h * DH, DH), DH), :] = (acc / l).astype(BF16)
            return carry

        jax.lax.fori_loop(0, H, head, 0)
        for c in range(nch):
            a_chunk(c)

    @pl.when(t == NQ - 1)
    def _():
        wait_out(row0)


@jax.jit
def pallas_concat_heads__softmax_full_mha__ssm_conv_s5__prompt_kernel(
    A_x: jax.Array,
    A_wqkv: jax.Array,
    A_wo: jax.Array,
    B_x: jax.Array,
    B_Lambda_re: jax.Array,
    B_Lambda_im: jax.Array,
    B_B_re: jax.Array,
    B_B_im: jax.Array,
    B_C_re: jax.Array,
    B_C_im: jax.Array,
    B_log_dt: jax.Array,
    B_Dskip: jax.Array,
):
    hbm = pl.BlockSpec(memory_space=pl.ANY)

    out = pl.pallas_call(
        _kernel,
        grid=(NQ,),
        in_specs=[hbm] * 12,
        out_specs=hbm,
        out_shape=jax.ShapeDtypeStruct((S, 2 * D), F32),
        scratch_shapes=[
            pltpu.VMEM((S, D), BF16),
            pltpu.VMEM((D, D), BF16),
            pltpu.VMEM((D, D), BF16),
            pltpu.VMEM((D, D), BF16),
            pltpu.VMEM((D, D), BF16),
            pltpu.VMEM((S, D), BF16),
            pltpu.VMEM((P, D), BF16),
            pltpu.VMEM((P, D), BF16),
            pltpu.VMEM((D, P), BF16),
            pltpu.VMEM((D, P), BF16),
            pltpu.SemaphoreType.DMA((16,)),
            pltpu.VMEM((D, S), BF16),
            pltpu.VMEM((4, S, 128), BF16),
            pltpu.VMEM((D, S), BF16),
            pltpu.VMEM((SKEW, KC, TQ), BF16),
            pltpu.VMEM((8, TQ), F32),
            pltpu.VMEM((max(len(PEND_KEYS), 1), 8, TQ), F32),
            pltpu.VMEM((8, TQ), F32),
            pltpu.VMEM((D, TQ), BF16),
            pltpu.VMEM((10, 8, P), F32),
            pltpu.VMEM((TQ, 2 * P), F32),
            pltpu.VMEM((2, 8, P), F32),
            pltpu.VMEM((P,), BF16),
            pltpu.VMEM((P,), BF16),
            pltpu.VMEM((P,), BF16),
            pltpu.VMEM((D,), BF16),
            pltpu.VMEM((TQ, 2 * D), F32),
            pltpu.SemaphoreType.DMA((2 * (TQ // RC),)),
            pltpu.VMEM((D, D), BF16),
            pltpu.VMEM((D, D), BF16),
            pltpu.VMEM((DH, TQ), F32),
            pltpu.VMEM((4, len(VPU_CHUNKS), VR, 128), F32),
            pltpu.VMEM((2, DH, TQ), F32),
        ],
        compiler_params=pltpu.CompilerParams(
            dimension_semantics=("arbitrary",),
            vmem_limit_bytes=100 * 1024 * 1024,
        ),
        name="mha_s5",
    )(A_x.reshape(S, D), A_wqkv, A_wo, B_x.reshape(S, D), B_Lambda_re, B_Lambda_im,
      B_B_re, B_B_im, B_C_re, B_C_im, B_log_dt, B_Dskip)
    return out.reshape(1, S, 2 * D)
```
